```python
import os as _os
_os.environ.setdefault("JAX_PLATFORMS", "cpu")
import jax
import jax.numpy as jnp

def _softmax(x, axis=-1):
    return jax.nn.softmax(x, axis=axis)
def _gelu(x):
    return jax.nn.gelu(x, approximate=True)
def _silu(x):
    return jax.nn.silu(x)
def _sigmoid(x):
    return jax.nn.sigmoid(x)
def _layernorm(x, axis=-1, eps=1e-5):
    m = jnp.mean(x, axis=axis, keepdims=True)
    v = jnp.var(x, axis=axis, keepdims=True)
    return (x - m) / jnp.sqrt(v + eps)
def _scatter_add(tgt, idx, src, axis=0):
    return tgt.at[idx].add(src)
def _segment_sum(src, seg, n):
    return jax.ops.segment_sum(src, seg, n)
class _Rng:
    def __init__(self, key):
        self._k = key
    def _next(self):
        self._k, sub = jax.random.split(self._k)
        return sub
    def normal(self, shape):
        return jax.random.normal(self._next(), shape, dtype=jnp.bfloat16)
    def randint(self, lo, hi, shape):
        return jax.random.randint(self._next(), shape, lo, hi, dtype=jnp.int32)
    def uniform(self, shape, lo=0.0, hi=1.0):
        return jax.random.uniform(self._next(), shape, jnp.bfloat16, lo, hi)
    def permutation(self, n):
        return jax.random.permutation(self._next(), n)


kernel_name = 'parallel_sum__softmax_full_mha__swiglu_ffn__prompt'

def setup_inputs():
    _rng = _Rng(jax.random.key(int.from_bytes(__import__("os").urandom(4), "little")))
    _w = (lambda a: (lambda t: t.astype(jnp.bfloat16) if jnp.issubdtype(t.dtype, jnp.floating) else t)(jnp.asarray(a)))
    def _A_setup():
        B, S, D = 1, 2048, 640
        return {
            "x": _w((lambda *s: _rng.normal(s) * 0.05)(B, S, D)),
            "wqkv": _w((lambda *s: _rng.normal(s) * 0.1)(D, 3 * D)),
            "wo": _w((lambda *s: _rng.normal(s) * 0.05)(D, D)),
        }
    _A_in = _A_setup()

    def _B_setup():
        B, S, D, F = 1, 2048, 640, 1536
        return {
            "x": _w((lambda *s: _rng.normal(s) * 0.05)(B, S, D)),
            "w_gate": _w((lambda *s: _rng.normal(s) * 0.05)(D, F)),
            "w_up": _w((lambda *s: _rng.normal(s) * 0.05)(D, F)),
            "w_down": _w((lambda *s: _rng.normal(s) * 0.05)(F, D)),
        }
    _B_in = _B_setup()

    return {
        "A_x": _A_in["x"],
        "A_wqkv": _A_in["wqkv"],
        "A_wo": _A_in["wo"],
        "B_x": _B_in["x"],
        "B_w_gate": _B_in["w_gate"],
        "B_w_up": _B_in["w_up"],
        "B_w_down": _B_in["w_down"],
    }

def reference(A_x, A_wqkv, A_wo, B_x, B_w_gate, B_w_up, B_w_down):
    def _A_ref(x, wqkv, wo):
        B, S, D = x.shape
        H = 32; Dh = D // H
        qkv = (lambda x, *d: x.transpose(*d))((x @ wqkv).reshape(B, S, 3, H, Dh), 2, 0, 3, 1, 4)
        q, k, v = qkv[0], qkv[1], qkv[2]
        scale = Dh ** -0.5
        scores = jnp.einsum("bhqd,bhkd->bhqk", q, k) * scale
        p = _softmax(scores, axis=-1)
        o = jnp.einsum("bhqk,bhkd->bhqd", p, v)
        return (lambda x, *d: x.transpose(*d))(o, 0, 2, 1, 3).reshape(B, S, D) @ wo

    def _B_ref(x, w_gate, w_up, w_down):
        g = _silu(x @ w_gate)
        u = x @ w_up
        return (g * u) @ w_down

    x = A_x
    xn = _layernorm(x, axis=-1)
    return x + _A_ref(xn, A_wqkv, A_wo) + _B_ref(xn, B_w_gate, B_w_up, B_w_down)
```

```python
import jax
import jax.numpy as jnp
import jax.experimental.pallas as pl
import jax.experimental.pallas.tpu as pltpu

CFG = dict(QT=512, RC=512, TC=256, CH=128, NI=4)
S, D, H, Dh, F = 2048, 640, 32, 20, 1536
VR = 24
LOG2E = 1.4426950408889634
f32, bf16 = jnp.float32, jnp.bfloat16


def dot(a, b):
    return jnp.dot(a, b, preferred_element_type=f32)


def kernel(x_hbm, wqkv_hbm, wo_hbm, wg_hbm, wu_hbm, wd_hbm, o_hbm,
           x_ref, wqkv_ref, wo_ref, wg_ref, wu_ref, wd_ref, ob_ref,
           xn_ref, kg_ref, qt_ref, vt_ref, ot_ref, s_refs, qm_ref, m_ref,
           x_sem, w_sem, o_sem):
    QT, RC, TC, CH, NI = (CFG[k] for k in ("QT", "RC", "TC", "CH", "NI"))
    NQ = S // QT
    NB = H * NQ // NI
    qscale = (Dh ** -0.5) * LOG2E

    def rows(c, n):
        return pl.ds(pl.multiple_of(c * n, n), n)

    def x_copy(c):
        return pltpu.make_async_copy(x_hbm.at[rows(c, RC)], x_ref.at[rows(c, RC)], x_sem.at[c])

    def wqkv_copy(j):
        c = pl.ds(j * D, D)
        return pltpu.make_async_copy(wqkv_hbm.at[:, c], wqkv_ref.at[:, c], w_sem.at[j])

    late = [pltpu.make_async_copy(h, v, w_sem.at[3 + j]) for j, (h, v) in enumerate(
        ((wg_hbm, wg_ref), (wu_hbm, wu_ref), (wd_hbm, wd_ref), (wo_hbm, wo_ref)))]

    def o_copy(c):
        return pltpu.make_async_copy(ob_ref.at[rows(c, TC)], o_hbm.at[rows(c, TC)], o_sem.at[c])

    NC = S // RC
    x_copy(0).start()
    wqkv_copy(0).start()
    wqkv_copy(1).start()
    wqkv_copy(2).start()
    for j in range(3):
        wqkv_copy(j).wait()
    for c in range(1, NC):
        x_copy(c).start()

    def proj(c, _):
        x_copy(c).wait()
        r = rows(c, RC)
        x = x_ref[r, :].astype(f32)
        xc = x - jnp.mean(x, axis=-1, keepdims=True)
        v = jnp.mean(xc * xc, axis=-1, keepdims=True)
        xn = (xc * jax.lax.rsqrt(v + 1e-5)).astype(bf16)
        xn_ref[r, :] = xn
        vt = dot(xn, wqkv_ref[:, 2 * D:3 * D]).T
        row = jax.lax.broadcasted_iota(jnp.int32, (VR - Dh, RC), 0)
        pad = jnp.where(row == 0, 1.0, 0.0).astype(f32)
        for h in range(H):
            vt_ref[h, :, r] = jnp.concatenate([vt[Dh * h:Dh * h + Dh], pad], axis=0)
        qt_ref[:, r] = (dot(xn, wqkv_ref[:, 0:D]) * qscale).T
        k = dot(xn, wqkv_ref[:, D:2 * D])
        for g in range(6):
            lo = min(120 * g, D - 128)
            kg_ref[g, r, :] = k[:, lo:lo + 128].astype(bf16)
        return 0

    jax.lax.fori_loop(0, NC, proj, 0)
    for cp in late:
        cp.start()

    def item(n, u):
        n = n * NI + u
        return n >> 3, (n >> 1) & 3, u % 2

    def group(i):
        return (i * 11) >> 5

    def prep_q(n, u):
        i, t, j = item(n, u)
        lo = jnp.minimum(120 * group(i), D - 128)
        qw = qt_ref[pl.ds(pl.multiple_of(lo, 8), 128), rows(t, QT)]
        row = jax.lax.broadcasted_iota(jnp.int32, (128, QT), 0) - (40 * i - lo + Dh * j)
        qm_ref[u] = jnp.where((row >= 0) & (row < Dh), qw, 0.0).astype(bf16)

    def block(n, do_qk, do_pv):
        prev = None
        for u in range(NI):
            s_ref = s_refs[u]
            mx = o = None
            if do_qk:
                g = group(item(n + 1, u)[0])
                qm = qm_ref[u]
            if do_pv:
                i, t, j = item(n, u)
                m = m_ref[u]
            for kc in range(0, S, CH):
                ks = slice(kc, kc + CH)
                if do_pv:
                    p = jnp.exp2(s_ref[ks, :].reshape(CH // 8, 8, QT) - m).reshape(CH, QT)
                if do_qk:
                    s = dot(kg_ref[g, ks, :], qm)
                    s_ref[ks, :] = s
                    cm = jnp.max(s.reshape(CH // 8, 8, QT), axis=0)
                    mx = cm if mx is None else jnp.maximum(mx, cm)
                if do_pv:
                    pv = dot(vt_ref[2 * i + j, :, ks], p)
                    o = pv if o is None else o + pv
            if do_qk:
                m_ref[u] = jnp.broadcast_to(jnp.max(mx, axis=0, keepdims=True), (8, QT))
                prep_q(jnp.minimum(n + 2, NB - 1), u)
            if do_pv:
                on = o[0:Dh] / o[Dh:Dh + 1]
                if j == 1:
                    ot_ref[pl.ds(pl.multiple_of(40 * i, 8), 40), rows(t, QT)] = jnp.concatenate([prev, on], axis=0)
                prev = on

    for u in range(NI):
        prep_q(0, u)
    block(-1, True, False)

    def body(n, _):
        block(n, True, True)
        return 0

    jax.lax.fori_loop(0, NB - 1, body, 0)

    for cp in late:
        cp.wait()

    block(NB - 1, False, True)

    def tail(c, _):
        r = rows(c, TC)
        xn = xn_ref[r, :]
        g = dot(xn, wg_ref[...])
        u = dot(xn, wu_ref[...])
        a = dot(ot_ref[:, r].T.astype(bf16), wo_ref[...])
        hmid = (g * jax.nn.sigmoid(g) * u).astype(bf16)
        y = dot(hmid, wd_ref[...])
        ob_ref[r, :] = (x_ref[r, :].astype(f32) + a + y).astype(ob_ref.dtype)
        o_copy(c).start()
        return 0

    jax.lax.fori_loop(0, S // TC, tail, 0)
    for c in range(S // TC):
        o_copy(c).wait()


@jax.jit
def pallas_parallel_sum__softmax_full_mha__swiglu_ffn__prompt_kernel(
        A_x, A_wqkv, A_wo, B_x, B_w_gate, B_w_up, B_w_down):
    QT, NI = CFG["QT"], CFG["NI"]
    hbm = pl.BlockSpec(memory_space=pl.ANY)
    out = pl.pallas_call(
        kernel,
        out_shape=jax.ShapeDtypeStruct((S, D), A_x.dtype),
        in_specs=[hbm] * 6,
        out_specs=hbm,
        scratch_shapes=[
            pltpu.VMEM((S, D), bf16),
            pltpu.VMEM((D, 3 * D), bf16),
            pltpu.VMEM((D, D), bf16),
            pltpu.VMEM((D, F), bf16),
            pltpu.VMEM((D, F), bf16),
            pltpu.VMEM((F, D), bf16),
            pltpu.VMEM((S, D), A_x.dtype),
            pltpu.VMEM((S, D), bf16),
            pltpu.VMEM((6, S, 128), bf16),
            pltpu.VMEM((D, S), f32),
            pltpu.VMEM((H, VR, S), f32),
            pltpu.VMEM((D, S), f32),
            [pltpu.VMEM((S, QT), f32) for _ in range(NI)],
            pltpu.VMEM((NI, 128, QT), bf16),
            pltpu.VMEM((NI, 8, QT), f32),
            pltpu.SemaphoreType.DMA((S // CFG["RC"],)),
            pltpu.SemaphoreType.DMA((7,)),
            pltpu.SemaphoreType.DMA((S // CFG["TC"],)),
        ],
        compiler_params=pltpu.CompilerParams(vmem_limit_bytes=112 * 1024 * 1024),
    )(A_x.reshape(S, D), A_wqkv, A_wo, B_w_gate, B_w_up, B_w_down)
    return out.reshape(A_x.shape)
```
